```python
import os as _os
_os.environ.setdefault("JAX_PLATFORMS", "cpu")
import jax
import jax.numpy as jnp

def _softmax(x, axis=-1):
    return jax.nn.softmax(x, axis=axis)
def _gelu(x):
    return jax.nn.gelu(x, approximate=True)
def _silu(x):
    return jax.nn.silu(x)
def _sigmoid(x):
    return jax.nn.sigmoid(x)
def _layernorm(x, axis=-1, eps=1e-5):
    m = jnp.mean(x, axis=axis, keepdims=True)
    v = jnp.var(x, axis=axis, keepdims=True)
    return (x - m) / jnp.sqrt(v + eps)
def _scatter_add(tgt, idx, src, axis=0):
    return tgt.at[idx].add(src)
def _segment_sum(src, seg, n):
    return jax.ops.segment_sum(src, seg, n)
class _Rng:
    def __init__(self, key):
        self._k = key
    def _next(self):
        self._k, sub = jax.random.split(self._k)
        return sub
    def normal(self, shape):
        return jax.random.normal(self._next(), shape, dtype=jnp.bfloat16)
    def randint(self, lo, hi, shape):
        return jax.random.randint(self._next(), shape, lo, hi, dtype=jnp.int32)
    def uniform(self, shape, lo=0.0, hi=1.0):
        return jax.random.uniform(self._next(), shape, jnp.bfloat16, lo, hi)
    def permutation(self, n):
        return jax.random.permutation(self._next(), n)


kernel_name = 'standalone__dcn_v2_cross__recsys'

def setup_inputs():
    _rng = _Rng(jax.random.key(int.from_bytes(__import__("os").urandom(4), "little")))
    _w = (lambda a: (lambda t: t.astype(jnp.bfloat16) if jnp.issubdtype(t.dtype, jnp.floating) else t)(jnp.asarray(a)))
    B, F, D, L = 4096, 26, 128, 6
    Din = min(F * D, 1024)
    return {
        "x0": _w((lambda *s: _rng.normal(s) * 0.05)(B, Din)),
        "ws": _w((lambda *s: _rng.normal(s) * 0.05)(L, Din, Din)),
        "bs": _w((lambda *s: _rng.normal(s) * 0.05)(L, Din)),
    }

def reference(x0, ws, bs):
    x = x0
    for l in range(ws.shape[0]):
        x = x0 * (x @ ws[l] + bs[l]) + x
    return x
```

```python
import jax, jax.numpy as jnp
from jax import lax
from jax.experimental import pallas as pl
from jax.experimental.pallas import tpu as pltpu

def _build(TM=512, P=512, vmem=100, cuts=(0, 256, 512, 1024), flags=None, allstart=0):
    def kern(x0_hbm, w_hbm, b_hbm, o_hbm, w_ref, b_ref, xp, sp, x_buf, o_buf, wsem, w0sem, bsem, psem, xsem, osem):
        L, D, _ = w_ref.shape
        NT = (x0_hbm.shape[0] - P) // TM
        H = P // 2
        nc = len(cuts) - 1
        def xcp(i, slot):
            return pltpu.make_async_copy(x0_hbm.at[pl.ds(P + i * TM, TM), :], x_buf.at[slot], xsem.at[slot])
        def ocp(i, slot):
            return pltpu.make_async_copy(o_buf.at[slot], o_hbm.at[pl.ds(P + i * TM, TM), :], osem.at[slot])
        def wcp(l):
            return pltpu.make_async_copy(w_hbm.at[l], w_ref.at[l], wsem.at[l])
        def w0cp(c):
            s = slice(cuts[c], cuts[c + 1])
            return pltpu.make_async_copy(w_hbm.at[0, :, s], w_ref.at[0, :, s], w0sem.at[c])
        def pcp(h):
            return pltpu.make_async_copy(x0_hbm.at[h * H:(h + 1) * H, :], xp.at[h * H:(h + 1) * H, :], psem.at[h])
        pout = pltpu.make_async_copy(sp, o_hbm.at[0:P, :], psem.at[2])
        bcp = pltpu.make_async_copy(b_hbm, b_ref, bsem)

        def cross(x0, x, acc, b):
            return (x0.astype(jnp.float32) * (acc + b.astype(jnp.float32)) + x.astype(jnp.float32)).astype(jnp.bfloat16)

        pcp(0).start(); w0cp(0).start(); bcp.start(); pcp(1).start()
        if allstart:
            for c in range(1, nc):
                w0cp(c).start()

        def first(r, c):
            s = slice(cuts[c], cuts[c + 1])
            acc = jnp.dot(xp[r, :], w_ref[0, :, s], preferred_element_type=jnp.float32)
            x0 = xp[r, s]
            sp[r, s] = cross(x0, x0, acc, b_ref[0:1, s])
        pcp(0).wait(); w0cp(0).wait(); bcp.wait()
        if not allstart and nc > 1:
            w0cp(1).start()
        first(slice(0, H), 0)
        pcp(1).wait()
        if nc == 1:
            wcp(1).start()
        first(slice(H, P), 0)
        for c in range(1, nc):
            w0cp(c).wait()
            if c + 1 < nc:
                if not allstart:
                    w0cp(c + 1).start()
            else:
                wcp(1).start()
            first(slice(0, P), c)

        def lbody(l, carry):
            wcp(l).wait()
            @pl.when(l + 1 < L)
            def _():
                wcp(l + 1).start()
            @pl.when(l + 1 == L)
            def _():
                xcp(0, 0).start()
            x = sp[...]
            acc = jnp.dot(x, w_ref[l], preferred_element_type=jnp.float32)
            bf = b_ref[...].astype(jnp.float32)
            rows = lax.broadcasted_iota(jnp.int32, bf.shape, 0)
            b = jnp.sum(jnp.where(rows == l, bf, 0.0), axis=0, keepdims=True)
            sp[...] = cross(xp[...], x, acc, b)
            return carry
        lax.fori_loop(1, L, lbody, 0)
        pout.start()

        def body(i, carry):
            slot = i % 2
            xcp(i, slot).wait()
            @pl.when(i + 1 < NT)
            def _():
                xcp(i + 1, 1 - slot).start()
            @pl.when(i >= 2)
            def _():
                ocp(i - 2, slot).wait()
            x = x_buf[slot]
            x0 = x
            for l in range(L):
                acc = jnp.dot(x, w_ref[l], preferred_element_type=jnp.float32)
                x = cross(x0, x, acc, b_ref[l:l + 1, :])
            o_buf[slot] = x
            ocp(i, slot).start()
            return carry
        lax.fori_loop(0, NT, body, 0)
        pout.wait()
        ocp(NT - 2, (NT - 2) % 2).wait()
        ocp(NT - 1, (NT - 1) % 2).wait()

    def f(x0, ws, bs):
        B, D = x0.shape; L = ws.shape[0]
        anyspec = pl.BlockSpec(memory_space=pl.ANY)
        return pl.pallas_call(kern,
            in_specs=[anyspec, anyspec, anyspec],
            out_specs=anyspec,
            out_shape=jax.ShapeDtypeStruct((B, D), x0.dtype),
            scratch_shapes=[pltpu.VMEM((L, D, D), jnp.bfloat16), pltpu.VMEM((L, D), jnp.bfloat16),
                            pltpu.VMEM((P, D), jnp.bfloat16), pltpu.VMEM((P, D), jnp.bfloat16),
                            pltpu.VMEM((2, TM, D), jnp.bfloat16), pltpu.VMEM((2, TM, D), jnp.bfloat16),
                            pltpu.SemaphoreType.DMA((L,)), pltpu.SemaphoreType.DMA((len(cuts) - 1,)), pltpu.SemaphoreType.DMA(()),
                            pltpu.SemaphoreType.DMA((3,)),
                            pltpu.SemaphoreType.DMA((2,)), pltpu.SemaphoreType.DMA((2,))],
            compiler_params=pltpu.CompilerParams(vmem_limit_bytes=vmem * 2**20, flags=flags),
        )(x0, ws, bs)
    return f


@jax.jit
def pallas_standalone__dcn_v2_cross__recsys_kernel(x0: jax.Array, ws: jax.Array, bs: jax.Array):
    return _build()(x0, ws, bs)
```
